```python
import os as _os
_os.environ.setdefault("JAX_PLATFORMS", "cpu")
import jax
import jax.numpy as jnp

def _softmax(x, axis=-1):
    return jax.nn.softmax(x, axis=axis)
def _gelu(x):
    return jax.nn.gelu(x, approximate=True)
def _silu(x):
    return jax.nn.silu(x)
def _sigmoid(x):
    return jax.nn.sigmoid(x)
def _layernorm(x, axis=-1, eps=1e-5):
    m = jnp.mean(x, axis=axis, keepdims=True)
    v = jnp.var(x, axis=axis, keepdims=True)
    return (x - m) / jnp.sqrt(v + eps)
def _scatter_add(tgt, idx, src, axis=0):
    return tgt.at[idx].add(src)
def _segment_sum(src, seg, n):
    return jax.ops.segment_sum(src, seg, n)
class _Rng:
    def __init__(self, key):
        self._k = key
    def _next(self):
        self._k, sub = jax.random.split(self._k)
        return sub
    def normal(self, shape):
        return jax.random.normal(self._next(), shape, dtype=jnp.bfloat16)
    def randint(self, lo, hi, shape):
        return jax.random.randint(self._next(), shape, lo, hi, dtype=jnp.int32)
    def uniform(self, shape, lo=0.0, hi=1.0):
        return jax.random.uniform(self._next(), shape, jnp.bfloat16, lo, hi)
    def permutation(self, n):
        return jax.random.permutation(self._next(), n)


kernel_name = 'sequential_preLN__linear_kernel_hedgehog__dense_activation_squared_relu__prompt'

def setup_inputs():
    _rng = _Rng(jax.random.key(int.from_bytes(__import__("os").urandom(4), "little")))
    _w = (lambda a: (lambda t: t.astype(jnp.bfloat16) if jnp.issubdtype(t.dtype, jnp.floating) else t)(jnp.asarray(a)))
    def _A_setup():
        B, S, D, H = 1, 2048, 512, 32
        Dh = D // H
        return {
            "x": _w((lambda *s: _rng.normal(s) * 0.05)(B, S, D)),
            "wqkv": _w((lambda *s: _rng.normal(s) * 0.2)(D, 3 * D)),
            "w_phi": _w((lambda *s: _rng.normal(s) * 0.2)(H, Dh, Dh) * (Dh ** -0.5)),
            "wo": _w((lambda *s: _rng.normal(s) * 0.05)(D, D)),
        }
    _A_in = _A_setup()

    def _B_setup():
        B, S, D, F = 1, 2048, 512, 1792
        return {
            "x": _w((lambda *s: _rng.normal(s) * 0.05)(B, S, D)),
            "w1": _w((lambda *s: _rng.normal(s) * 0.05)(D, F)),
            "b1": _w((lambda *s: _rng.normal(s) * 0.05)(F)),
            "w2": _w((lambda *s: _rng.normal(s) * 0.05)(F, D)),
            "b2": _w((lambda *s: _rng.normal(s) * 0.05)(D)),
        }
    _B_in = _B_setup()

    return {
        "A_x": _A_in["x"],
        "A_wqkv": _A_in["wqkv"],
        "A_w_phi": _A_in["w_phi"],
        "A_wo": _A_in["wo"],
        "B_x": _B_in["x"],
        "B_w1": _B_in["w1"],
        "B_b1": _B_in["b1"],
        "B_w2": _B_in["w2"],
        "B_b2": _B_in["b2"],
    }

def reference(A_x, A_wqkv, A_w_phi, A_wo, B_x, B_w1, B_b1, B_w2, B_b2):
    def _A_ref(x, wqkv, w_phi, wo):
        B, S, D = x.shape
        H = 32; Dh = D // H
        qkv = (lambda x, *d: x.transpose(*d))((x @ wqkv).reshape(B, S, 3, H, Dh), 2, 0, 3, 1, 4)
        q, k, v = qkv[0], qkv[1], qkv[2]
        pq = jnp.einsum("bhsd,hdf->bhsf", q, w_phi)
        pk = jnp.einsum("bhsd,hdf->bhsf", k, w_phi)
        phi_q = jnp.concatenate([_softmax(pq, axis=-1), _softmax(-pq, axis=-1)], axis=-1)
        phi_k = jnp.concatenate([_softmax(pk, axis=-1), _softmax(-pk, axis=-1)], axis=-1)
        kv = jnp.einsum("bhsf,bhsd->bhfd", phi_k, v)
        z  = jnp.einsum("bhsf->bhf", phi_k)
        num = jnp.einsum("bhqf,bhfd->bhqd", phi_q, kv)
        den = jnp.einsum("bhqf,bhf->bhq", phi_q, z)[..., None] + 1e-6
        o = num / den
        return (lambda x, *d: x.transpose(*d))(o, 0, 2, 1, 3).reshape(B, S, D) @ wo

    def _B_ref(x, w1, b1, w2, b2):
        h = jnp.einsum("bsd,df->bsf", x, w1) + b1
        zero = jnp.zeros_like(h)
        r = jnp.where(h > zero, h, zero)
        h = r * r
        out = jnp.einsum("bsf,fd->bsd", h, w2) + b2
        return out

    x = A_x
    h = x + _A_ref(_layernorm(x, axis=-1), A_wqkv, A_w_phi, A_wo)
    h2 = h + _B_ref(_layernorm(h, axis=-1), B_w1, B_b1, B_w2, B_b2)
    return h2
```

```python
import functools
import math

import jax
import jax.numpy as jnp
from jax import lax
import jax.experimental.pallas as pl
import jax.experimental.pallas.tpu as pltpu

_LOG2E = math.log2(math.e)
_NT = (((1,), (1,)), ((), ()))
_NN = (((1,), (0,)), ((), ()))


def _dot(a, b, dims=_NN):
    return lax.dot_general(a, b, dims, preferred_element_type=jnp.float32)


def _recip(x):
    return pl.reciprocal(x, full_range=False)


def _layernorm(x):
    m = jnp.mean(x, axis=-1, keepdims=True)
    xc = x - m
    v = jnp.mean(xc * xc, axis=-1, keepdims=True)
    return xc * lax.rsqrt(v + 1e-5)


def _allred(op, rows):
    r = functools.reduce(op, rows)
    return op(r, pltpu.roll(r, 4, 0))


def _dual_softmax(p):
    rows = [p[m * 8:(m + 1) * 8] for m in range(8)]
    mx = _allred(jnp.maximum, rows)
    mn = _allred(jnp.minimum, rows)
    ep = [jnp.exp2(r - mx) for r in rows]
    en = [jnp.exp2(mn - r) for r in rows]
    rp = _recip(_allred(jnp.add, ep))
    rn = _recip(_allred(jnp.add, en))
    return [e * rp for e in ep] + [e * rn for e in en]


@jax.jit
def pallas_sequential_preLN__linear_kernel_hedgehog__dense_activation_squared_relu__prompt_kernel(
    A_x, A_wqkv, A_w_phi, A_wo, B_x, B_w1, B_b1, B_w2, B_b2,
):
    B, S, D = A_x.shape
    H, Dh, _ = A_w_phi.shape
    F = B_w1.shape[1]
    G = D // 128
    G4 = 2 * G
    SB = 512
    NB = S // SB
    bf16, f32 = jnp.bfloat16, jnp.float32

    def kernel(x_hbm, wqkv_hbm, wphi_hbm, wo_hbm, w1_hbm, b1_hbm, w2_hbm, b2_hbm, o_ref,
               x_v, wqkv_v, wphi_v, wo_v, w1_v, b1_v, w2_v, b2_v,
               wT, phiq, kvacc, zacc, kvT, zb, sems):
        ph = pl.program_id(0)
        i = pl.program_id(1)

        def cp(src, dst, k):
            return pltpu.make_async_copy(src, dst, sems.at[k])

        def cp_x(b):
            return cp(x_hbm.at[pl.ds(b * SB, SB)], x_v.at[pl.ds(b * SB, SB)], b)

        def cp_w(t):
            return cp(wqkv_hbm.at[:, pl.ds(t * D, D)], wqkv_v.at[:, pl.ds(t * D, D)], NB + t)

        cp_phi = cp(wphi_hbm, wphi_v, NB + 3)
        late = [cp(wo_hbm, wo_v, NB + 4), cp(w1_hbm, w1_v, NB + 5), cp(b1_hbm, b1_v, NB + 6),
                cp(w2_hbm, w2_v, NB + 7), cp(b2_hbm, b2_v, NB + 8)]

        @pl.when((ph == 0) & (i == 0))
        def _():
            cp_phi.start()
            cp_w(1).start()
            cp_x(0).start()
            cp_w(2).start()
            cp_w(0).start()
            for b in range(1, NB):
                cp_x(b).start()
            for c in late:
                c.start()
            cp_phi.wait()
            t2 = wphi_v[...]
            r0 = lax.broadcasted_iota(jnp.int32, (H, D), 0)
            c0 = lax.broadcasted_iota(jnp.int32, (H, D), 1)
            R = (r0 == c0 // Dh).astype(bf16)
            o1 = _dot(t2, R)
            r1 = lax.broadcasted_iota(jnp.int32, (Dh * Dh, D), 0)
            c1 = lax.broadcasted_iota(jnp.int32, (Dh * Dh, D), 1)
            o1 = jnp.where(r1 // Dh == c1 % Dh, o1, 0.0).astype(bf16)
            r2 = lax.broadcasted_iota(jnp.int32, (128, Dh * Dh), 0)
            c2 = lax.broadcasted_iota(jnp.int32, (128, Dh * Dh), 1)
            QT = ((r2 % 64) // 4 == c2 % Dh).astype(bf16)
            o2 = _dot(QT, o1)
            r3 = lax.broadcasted_iota(jnp.int32, (128, D), 0)
            c3 = lax.broadcasted_iota(jnp.int32, (128, D), 1)
            bdt = jnp.where((r3 // 64) * 4 + r3 % 4 == (c3 % 128) // Dh, o2, 0.0).astype(bf16)
            re = lax.broadcasted_iota(jnp.int32, (128, 128), 0)
            ce = lax.broadcasted_iota(jnp.int32, (128, 128), 1)
            eye = (re == ce).astype(bf16)
            for t in (1, 2, 0):
                cp_w(t).wait()
                for g in range(G):
                    w = wqkv_v[:, t * D + g * 128: t * D + (g + 1) * 128]
                    if t == 2:
                        wt = _dot(eye, w, _NT)
                    else:
                        wt = _dot(bdt[:, g * 128:(g + 1) * 128], w, _NT) * _LOG2E
                    wT[t * D + g * 128: t * D + (g + 1) * 128, :] = wt.astype(bf16)
            kvacc[...] = jnp.zeros_like(kvacc)
            zacc[...] = jnp.zeros_like(zacc)

        @pl.when(ph == 0)
        def _():
            for b in range(NB):
                @pl.when(i == b)
                def _():
                    cp_x(b).wait()
            rows = pl.ds(pl.multiple_of(i * SB, SB), SB)
            xn = _layernorm(x_v[rows, :].astype(f32)).astype(bf16)
            for g in range(G):
                pk = _dot(wT[D + g * 128: D + (g + 1) * 128, :], xn, _NT)
                vT = _dot(wT[2 * D + g * 128: 2 * D + (g + 1) * 128, :], xn, _NT).astype(bf16)
                for hf in range(2):
                    g4 = 2 * g + hf
                    phik = _dual_softmax(pk[hf * 64:(hf + 1) * 64])
                    zs = [functools.reduce(jnp.add, [r[:, j * 128:(j + 1) * 128] for j in range(SB // 128)])
                          for r in phik]
                    zacc[g4] += jnp.concatenate(zs, axis=0)
                    phik_b = jnp.concatenate(phik, axis=0).astype(bf16)
                    kvacc[g4] += _dot(vT[hf * 64:(hf + 1) * 64], phik_b, _NT)
            for g in range(G):
                pq = _dot(wT[g * 128:(g + 1) * 128, :], xn, _NT)
                for hf in range(2):
                    phq = _dual_softmax(pq[hf * 64:(hf + 1) * 64])
                    phiq[2 * g + hf, :, rows] = jnp.concatenate(phq, axis=0).astype(bf16)

        @pl.when((ph == 1) & (i == 0))
        def _():
            for c in late:
                c.wait()
            r2 = lax.broadcasted_iota(jnp.int32, (64, 128), 0)
            c2 = lax.broadcasted_iota(jnp.int32, (64, 128), 1)
            kmask = (r2 // Dh) == (c2 % 4)
            for g4 in range(G4):
                kvT[g4] = jnp.where(kmask, kvacc[g4], 0.0).astype(bf16)
                z = jnp.sum(zacc[g4], axis=-1, keepdims=True)
                zb[g4] = jnp.broadcast_to(z, (128, 128))

        @pl.when(ph == 1)
        def _():
            rows = pl.ds(pl.multiple_of(i * SB, SB), SB)
            os_ = []
            for g in range(G):
                parts = []
                for hf in range(2):
                    g4 = 2 * g + hf
                    pq = phiq[g4, :, rows]
                    numT = _dot(kvT[g4], pq)
                    pqf = pq.astype(f32)
                    zg = zb[g4]
                    den = None
                    for r in range(16):
                        zr = zg[r * 8:(r + 1) * 8]
                        t = pqf[r * 8:(r + 1) * 8] * jnp.concatenate([zr] * (SB // 128), axis=1)
                        den = t if den is None else den + t
                    den = den + pltpu.roll(den, 4, 0)
                    rd = _recip(den + 1e-6)
                    for h in range(4):
                        parts.append(numT[h * Dh:(h + 1) * Dh] * jnp.broadcast_to(rd[h:h + 1], (Dh, SB)))
                oT = jnp.concatenate(parts, axis=0)
                os_.append(oT.astype(bf16).T)
            o = jnp.concatenate(os_, axis=1)
            h = x_v[rows, :].astype(f32) + _dot(o, wo_v[...])
            hn = _layernorm(h).astype(bf16)
            a = _dot(hn, w1_v[...]) + b1_v[...].astype(f32).reshape(1, F)
            a = jnp.maximum(a, 0.0)
            a = (a * a).astype(bf16)
            out = h + _dot(a, w2_v[...]) + b2_v[...].astype(f32).reshape(1, D)
            o_ref[...] = out.astype(o_ref.dtype)

    x2 = A_x.reshape(S, D)
    wphi2 = jnp.transpose(A_w_phi, (1, 2, 0)).reshape(Dh * Dh, H)
    any_spec = pl.BlockSpec(memory_space=pl.ANY)
    out = pl.pallas_call(
        kernel,
        grid=(2, NB),
        in_specs=[any_spec] * 8,
        out_specs=pl.BlockSpec((SB, D), lambda p, i: (p * i, 0)),
        out_shape=jax.ShapeDtypeStruct((S, D), A_x.dtype),
        scratch_shapes=[
            pltpu.VMEM((S, D), bf16),
            pltpu.VMEM((D, 3 * D), bf16),
            pltpu.VMEM((Dh * Dh, H), bf16),
            pltpu.VMEM((D, D), bf16),
            pltpu.VMEM((D, F), bf16),
            pltpu.VMEM((F,), bf16),
            pltpu.VMEM((F, D), bf16),
            pltpu.VMEM((D,), bf16),
            pltpu.VMEM((3 * D, D), bf16),
            pltpu.VMEM((G4, 128, S), bf16),
            pltpu.VMEM((G4, 64, 128), f32),
            pltpu.VMEM((G4, 128, 128), f32),
            pltpu.VMEM((G4, 64, 128), bf16),
            pltpu.VMEM((G4, 128, 128), f32),
            pltpu.SemaphoreType.DMA((NB + 9,)),
        ],
        compiler_params=pltpu.CompilerParams(
            dimension_semantics=("arbitrary", "arbitrary"),
            vmem_limit_bytes=100 * 1024 * 1024,
        ),
    )(x2, A_wqkv, wphi2, A_wo, B_w1, B_b1, B_w2, B_b2)
    return out.reshape(B, S, D)
```

```python
import functools
import math

import jax
import jax.numpy as jnp
from jax import lax
import jax.experimental.pallas as pl
import jax.experimental.pallas.tpu as pltpu

_LOG2E = math.log2(math.e)
_NT = (((1,), (1,)), ((), ()))
_NN = (((1,), (0,)), ((), ()))


def _dot(a, b, dims=_NN):
    return lax.dot_general(a, b, dims, preferred_element_type=jnp.float32)


def _pk(x):
    return pltpu.bitcast(x, jnp.int32)


def _upk(x):
    return pltpu.bitcast(x, jnp.bfloat16)


def _recip(x):
    return pl.reciprocal(x, full_range=False)


def _layernorm(x):
    m = jnp.mean(x, axis=-1, keepdims=True)
    xc = x - m
    v = jnp.mean(xc * xc, axis=-1, keepdims=True)
    return xc * lax.rsqrt(v + 1e-5)


def _allred(op, rows):
    r = functools.reduce(op, rows)
    return op(r, pltpu.roll(r, 4, 0))


def _dual_softmax(p):
    rows = [p[m * 8:(m + 1) * 8] for m in range(8)]
    mx = _allred(jnp.maximum, rows)
    mn = _allred(jnp.minimum, rows)
    ep = [jnp.exp2(r - mx) for r in rows]
    en = [jnp.exp2(mn - r) for r in rows]
    rp = _recip(_allred(jnp.add, ep))
    rn = _recip(_allred(jnp.add, en))
    return [e * rp for e in ep] + [e * rn for e in en]


def _pack_feat(phi):
    return jnp.concatenate(
        [pltpu.pack_elementwise([phi[m], phi[8 + m]], packed_dtype=jnp.bfloat16) for m in range(8)], axis=0)


@jax.jit
def pallas_sequential_preLN__linear_kernel_hedgehog__dense_activation_squared_relu__prompt_kernel(
    A_x, A_wqkv, A_w_phi, A_wo, B_x, B_w1, B_b1, B_w2, B_b2,
):
    B, S, D = A_x.shape
    H, Dh, _ = A_w_phi.shape
    F = B_w1.shape[1]
    G = D // 128
    G4 = 2 * G
    SB = 512
    NB = S // SB
    NC0 = 32
    NC1 = 16
    SPLIT = 512
    R1A = (1, 2)
    R1B = (3,)
    NO = 4
    bf16, f32, i32 = jnp.bfloat16, jnp.float32, jnp.int32

    def kernel(x_hbm, wqkv_hbm, wphi_hbm, wo_hbm, w1_hbm, b1_hbm, w2_hbm, b2_hbm, o_hbm,
               x_v, wqkv_v, wphi_v, wo_v, w1_v, b1_v, w2_v, b2_v, o_v,
               wT, xn_c, xn_n, h_v, phiq, kvacc, zacc, kvT, zb, sems):
        s = pl.program_id(0)
        hn_c, hn_n = xn_c, xn_n

        def rows_of(i, c=0, n=SB):
            start = i * SB + c * n
            if not isinstance(start, int):
                start = pl.multiple_of(start, n)
            return pl.ds(start, n)

        def cp(src, dst, k):
            return pltpu.make_async_copy(src, dst, sems.at[k])

        def cp_x(b):
            return cp(x_hbm.at[pl.ds(b * SB, SB)], x_v.at[pl.ds(b * SB, SB)], b)

        def cp_w(t):
            return cp(wqkv_hbm.at[:, pl.ds(t * D, D)], wqkv_v.at[:, pl.ds(t * D, D)], NB + t)

        cp_phi = cp(wphi_hbm, wphi_v, NB + 3)
        late = [cp(wo_hbm, wo_v, NB + 4), cp(w1_hbm, w1_v, NB + 5), cp(b1_hbm, b1_v, NB + 6),
                cp(w2_hbm, w2_v, NB + 7), cp(b2_hbm, b2_v, NB + 8)]

        def cp_o(b, c=0, n=SB, k=None):
            r = rows_of(b, c, n)
            return cp(o_v.at[r], o_hbm.at[r], NB + 9 + (b if k is None else k))

        def build_bdt():
            t2 = wphi_v[...]
            r0 = lax.broadcasted_iota(i32, (H, D), 0)
            c0 = lax.broadcasted_iota(i32, (H, D), 1)
            o1 = _dot(t2, (r0 == c0 // Dh).astype(bf16))
            r1 = lax.broadcasted_iota(i32, (Dh * Dh, D), 0)
            c1 = lax.broadcasted_iota(i32, (Dh * Dh, D), 1)
            o1 = jnp.where(r1 // Dh == c1 % Dh, o1, 0.0).astype(bf16)
            r2 = lax.broadcasted_iota(i32, (128, Dh * Dh), 0)
            c2 = lax.broadcasted_iota(i32, (128, Dh * Dh), 1)
            o2 = _dot(((r2 % 64) // 4 == c2 % Dh).astype(bf16), o1)
            r3 = lax.broadcasted_iota(i32, (128, D), 0)
            c3 = lax.broadcasted_iota(i32, (128, D), 1)
            return jnp.where((r3 // 64) * 4 + r3 % 4 == (c3 % 128) // Dh, o2, 0.0).astype(bf16)

        def fold(t, bdt):
            for g in range(G):
                w = wqkv_v[:, t * D + g * 128: t * D + (g + 1) * 128]
                if bdt is None:
                    wt = w.T
                else:
                    wt = (_dot(bdt[:, g * 128:(g + 1) * 128], w, _NT) * _LOG2E).astype(bf16)
                wT[(t * D + g * 128) // 2:(t * D + (g + 1) * 128) // 2, :] = _pk(wt)

        def ln_x(i, dst):
            n = SB // NC0
            for c in range(NC0):
                dst[c * n // 2:(c + 1) * n // 2, :] = _pk(
                    _layernorm(x_v[rows_of(i, c, n), :].astype(f32)).astype(bf16))

        def proj(t, g):
            w = _upk(wT[(t * D + g * 128) // 2:(t * D + (g + 1) * 128) // 2, :])
            return _dot(w, _upk(xn_c[...]), _NT)

        def do_k(first, groups=range(G)):
            phiks = []
            for g in groups:
                pk = proj(1, g)
                for hf in range(2):
                    g4 = 2 * g + hf
                    phik = _dual_softmax(pk[hf * 64:(hf + 1) * 64])
                    zs = jnp.concatenate(
                        [functools.reduce(jnp.add, [r[:, j * 128:(j + 1) * 128] for j in range(SB // 128)])
                         for r in phik], axis=0)
                    zacc[g4] = zs if first else zacc[g4] + zs
                    phiks.append(_upk(_pack_feat(phik)))
            return phiks

        def do_q(i, groups=range(G)):
            for g in groups:
                pq = proj(0, g)
                for hf in range(2):
                    phiq[2 * g + hf, :, rows_of(i)] = _pack_feat(_dual_softmax(pq[hf * 64:(hf + 1) * 64]))

        def do_vkv(phiks, first):
            vTs = []
            for g in range(G):
                vT = proj(2, g)
                vTs += [vT[hf * 64:(hf + 1) * 64].astype(bf16) for hf in range(2)]
            for g4 in range(G4):
                kv = _dot(vTs[g4], phiks[g4], _NT)
                kvacc[g4] = kv if first else kvacc[g4] + kv

        def finalize():
            r2 = lax.broadcasted_iota(i32, (64, 128), 0)
            c2 = lax.broadcasted_iota(i32, (64, 128), 1)
            kmask = (r2 // Dh) == ((c2 // 2) % 4)
            for g4 in range(G4):
                kvT[g4] = _pk(jnp.where(kmask, kvacc[g4], 0.0).astype(bf16))
                z = jnp.sum(zacc[g4], axis=-1, keepdims=True)
                zb[g4] = jnp.broadcast_to(z, (128, 128))

        def attn_o(i):
            os_ = []
            for g in range(G):
                parts = []
                for hf in range(2):
                    g4 = 2 * g + hf
                    pqi = phiq[g4, :, rows_of(i)]
                    numT = _dot(_upk(kvT[g4]), _upk(pqi))
                    zg = zb[g4]
                    den = None
                    for r in range(16):
                        m, pn = r % 8, r // 8
                        pf = pltpu.unpack_elementwise(pqi[m * 8:(m + 1) * 8], index=pn,
                                                      packed_dtype=bf16, unpacked_dtype=f32)
                        t = pf * jnp.concatenate([zg[r * 8:(r + 1) * 8]] * (SB // 128), axis=1)
                        den = t if den is None else den + t
                    den = den + pltpu.roll(den, 4, 0)
                    rd = _recip(den + 1e-6)
                    for h in range(4):
                        parts.append(numT[h * Dh:(h + 1) * Dh] * jnp.broadcast_to(rd[h:h + 1], (Dh, SB)))
                oT = jnp.concatenate(parts, axis=0)
                os_.append(oT.astype(bf16).T)
            return jnp.concatenate(os_, axis=1)

        def attn_out(i, o, hn_dst):
            h_v[rows_of(i), :] = x_v[rows_of(i), :].astype(f32) + _dot(o, wo_v[...])
            n = SB // NC1
            for c in range(NC1):
                hn_dst[c * n // 2:(c + 1) * n // 2, :] = _pk(
                    _layernorm(h_v[rows_of(i, c, n), :]).astype(bf16))

        def ffn1(lo, hi):
            a = _dot(_upk(hn_c[...]), w1_v[:, lo:hi]) + b1_v[lo:hi].astype(f32).reshape(1, hi - lo)
            a = jnp.maximum(a, 0.0)
            return (a * a).astype(bf16)

        def ffn2(i, a, c=0, n=SB):
            r = rows_of(i, c, n)
            out = h_v[r, :] + _dot(a, w2_v[...]) + b2_v[...].astype(f32).reshape(1, D)
            o_v[r, :] = out.astype(o_v.dtype)

        @pl.when(s == 0)
        def _():
            cp_phi.start()
            cp_w(1).start()
            cp_x(0).start()
            cp_w(2).start()
            cp_x(1).start()
            cp_w(0).start()
            for b in range(2, NB):
                cp_x(b).start()
            for c in late:
                c.start()
            cp_phi.wait()
            bdt = build_bdt()
            cp_w(1).wait()
            fold(1, bdt)
            cp_x(0).wait()
            ln_x(0, xn_c)
            phiks = do_k(True)
            cp_w(2).wait()
            cp_x(1).wait()
            cp_w(0).wait()
            fold(0, bdt)
            fold(2, None)
            do_q(0)
            do_vkv(phiks, True)
            ln_x(1, xn_n)
            xn_c[...] = xn_n[...]

        @pl.when((s > 0) & (s < NB - 1))
        def _():
            for b in range(2, NB):
                @pl.when(s + 1 == b)
                def _():
                    cp_x(b).wait()
            phiks = do_k(False)
            do_q(s)
            do_vkv(phiks, False)
            ln_x(s + 1, xn_n)
            xn_c[...] = xn_n[...]

        @pl.when(s == NB - 1)
        def _():
            for c in late:
                c.wait()
            phiks = do_k(False)
            do_vkv(phiks, False)
            do_q(NB - 1, (0,))
            finalize()
            o = attn_o(0)
            do_q(NB - 1, R1A)
            attn_out(0, o, hn_n)
            do_q(NB - 1, R1B)
            hn_c[...] = hn_n[...]

        @pl.when((s >= NB) & (s < 2 * NB - 1))
        def _():
            i = s - NB
            o = attn_o(i + 1)
            a0 = ffn1(0, SPLIT)
            attn_out(i + 1, o, hn_n)
            a1 = ffn1(SPLIT, F)
            ffn2(i, jnp.concatenate([a0, a1], axis=1))
            hn_c[...] = hn_n[...]
            for b in range(NB - 1):
                @pl.when(i == b)
                def _():
                    cp_o(b).start()

        @pl.when(s == 2 * NB - 1)
        def _():
            a = ffn1(0, F)
            n = SB // NO
            for c in range(NO):
                ffn2(NB - 1, a[c * n:(c + 1) * n], c, n)
                cp_o(NB - 1, c, n, NB - 1 + c).start()
            for b in range(NB - 1):
                cp_o(b).wait()
            for c in range(NO):
                cp_o(NB - 1, c, n, NB - 1 + c).wait()

    x2 = A_x.reshape(S, D)
    wphi2 = jnp.transpose(A_w_phi, (1, 2, 0)).reshape(Dh * Dh, H)
    any_spec = pl.BlockSpec(memory_space=pl.ANY)
    out = pl.pallas_call(
        kernel,
        grid=(2 * NB,),
        in_specs=[any_spec] * 8,
        out_specs=any_spec,
        out_shape=jax.ShapeDtypeStruct((S, D), A_x.dtype),
        scratch_shapes=[
            pltpu.VMEM((S, D), bf16),
            pltpu.VMEM((D, 3 * D), bf16),
            pltpu.VMEM((Dh * Dh, H), bf16),
            pltpu.VMEM((D, D), bf16),
            pltpu.VMEM((D, F), bf16),
            pltpu.VMEM((F,), bf16),
            pltpu.VMEM((F, D), bf16),
            pltpu.VMEM((D,), bf16),
            pltpu.VMEM((S, D), bf16),
            pltpu.VMEM((3 * D // 2, D), i32),
            pltpu.VMEM((SB // 2, D), i32),
            pltpu.VMEM((SB // 2, D), i32),
            pltpu.VMEM((S, D), f32),
            pltpu.VMEM((G4, 64, S), i32),
            pltpu.VMEM((G4, 64, 128), f32),
            pltpu.VMEM((G4, 128, 128), f32),
            pltpu.VMEM((G4, 32, 128), i32),
            pltpu.VMEM((G4, 128, 128), f32),
            pltpu.SemaphoreType.DMA((NB + 9 + NB - 1 + NO,)),
        ],
        compiler_params=pltpu.CompilerParams(
            dimension_semantics=("arbitrary",),
            vmem_limit_bytes=100 * 1024 * 1024,
        ),
    )(x2, A_wqkv, wphi2, A_wo, B_w1, B_b1, B_w2, B_b2)
    return out.reshape(B, S, D)
```

```python
import functools
import math

import jax
import jax.numpy as jnp
from jax import lax
import jax.experimental.pallas as pl
import jax.experimental.pallas.tpu as pltpu

_LOG2E = math.log2(math.e)
_NT = (((1,), (1,)), ((), ()))
_NN = (((1,), (0,)), ((), ()))


def _dot(a, b, dims=_NN):
    return lax.dot_general(a, b, dims, preferred_element_type=jnp.float32)


def _pk(x):
    return pltpu.bitcast(x, jnp.int32)


def _upk(x):
    return pltpu.bitcast(x, jnp.bfloat16)


def _recip(x):
    return pl.reciprocal(x, full_range=False)


def _layernorm(x):
    m = jnp.mean(x, axis=-1, keepdims=True)
    xc = x - m
    v = jnp.mean(xc * xc, axis=-1, keepdims=True)
    return xc * lax.rsqrt(v + 1e-5)


def _allred(op, rows):
    r = functools.reduce(op, rows)
    return op(r, pltpu.roll(r, 4, 0))


def _dual_softmax(p):
    rows = [p[m * 8:(m + 1) * 8] for m in range(8)]
    mx = _allred(jnp.maximum, rows)
    mn = _allred(jnp.minimum, rows)
    ep = [jnp.exp2(r - mx) for r in rows]
    en = [jnp.exp2(mn - r) for r in rows]
    rp = _recip(_allred(jnp.add, ep))
    rn = _recip(_allred(jnp.add, en))
    return [e * rp for e in ep] + [e * rn for e in en]


def _pack_feat(phi):
    return jnp.concatenate(
        [pltpu.pack_elementwise([phi[m], phi[8 + m]], packed_dtype=jnp.bfloat16) for m in range(8)], axis=0)


@jax.jit
def pallas_sequential_preLN__linear_kernel_hedgehog__dense_activation_squared_relu__prompt_kernel(
    A_x, A_wqkv, A_w_phi, A_wo, B_x, B_w1, B_b1, B_w2, B_b2,
):
    B, S, D = A_x.shape
    H, Dh, _ = A_w_phi.shape
    F = B_w1.shape[1]
    G = D // 128
    G4 = 2 * G
    SB = 512
    NB = S // SB
    NCH = 32
    NO = 8
    assert B == 1 and Dh == 16 and D == H * Dh and D % 128 == 0 and S % SB == 0 and NB >= 3
    bf16, f32, i32 = jnp.bfloat16, jnp.float32, jnp.int32

    def kernel(x_hbm, wqkv_hbm, wphi_hbm, wo_hbm, w1_hbm, b1_hbm, w2_hbm, b2_hbm, o_hbm,
               x_v, wqkv_v, wphi_v, wo_v, w1_v, b1_v, w2_v, b2_v, o_v,
               wT, xn_c, xn_n, h_v, phiq, kvacc, zacc, kvT, zb, sems):
        s = pl.program_id(0)
        hn_c, hn_n = xn_c, xn_n

        def rows_of(i, c=0, n=SB):
            start = i * SB + c * n
            if not isinstance(start, int):
                start = pl.multiple_of(start, n)
            return pl.ds(start, n)

        def cp(src, dst, k):
            return pltpu.make_async_copy(src, dst, sems.at[k])

        SEM_PHI, SEM_X0A, SEM_WK0, SEM_A, SEM_WQ, SEM_B, SEM_C, SEM_D, SEM_OUT = range(9)

        def cp_x(b):
            r = pl.ds(b * SB, SB)
            return cp(x_hbm.at[r], x_v.at[r], SEM_B if b == 1 else SEM_C)

        def cp_x0(hf):
            r = pl.ds(hf * (SB // 2), SB // 2)
            return cp(x_hbm.at[r], x_v.at[r], (SEM_X0A, SEM_A)[hf])

        def cp_w(t):
            c = pl.ds(t * D, D)
            return cp(wqkv_hbm.at[:, c], wqkv_v.at[:, c], (SEM_WQ, None, SEM_B)[t])

        def cp_wk(hf):
            c = pl.ds(D + hf * (D // 2), D // 2)
            return cp(wqkv_hbm.at[:, c], wqkv_v.at[:, c], (SEM_WK0, SEM_A)[hf])

        cp_phi = cp(wphi_hbm, wphi_v, SEM_PHI)
        late = [cp(wo_hbm, wo_v, SEM_C), cp(w1_hbm, w1_v, SEM_D), cp(b1_hbm, b1_v, SEM_D),
                cp(w2_hbm, w2_v, SEM_D), cp(b2_hbm, b2_v, SEM_D)]

        def cp_o(b, c=0, n=SB):
            r = rows_of(b, c, n)
            return cp(o_v.at[r], o_hbm.at[r], SEM_OUT)

        def build_bdt():
            t2 = wphi_v[...]
            r0 = lax.broadcasted_iota(i32, (H, D), 0)
            c0 = lax.broadcasted_iota(i32, (H, D), 1)
            o1 = _dot(t2, (r0 == c0 // Dh).astype(bf16))
            r1 = lax.broadcasted_iota(i32, (Dh * Dh, D), 0)
            c1 = lax.broadcasted_iota(i32, (Dh * Dh, D), 1)
            o1 = jnp.where(r1 // Dh == c1 % Dh, o1, 0.0).astype(bf16)
            r2 = lax.broadcasted_iota(i32, (128, Dh * Dh), 0)
            c2 = lax.broadcasted_iota(i32, (128, Dh * Dh), 1)
            o2 = _dot(((r2 % 64) // 4 == c2 % Dh).astype(bf16), o1)
            r3 = lax.broadcasted_iota(i32, (128, D), 0)
            c3 = lax.broadcasted_iota(i32, (128, D), 1)
            return jnp.where((r3 // 64) * 4 + r3 % 4 == (c3 % 128) // Dh, o2, 0.0).astype(bf16)

        def fold(t, bdt, groups=range(G)):
            for g in groups:
                w = wqkv_v[:, t * D + g * 128: t * D + (g + 1) * 128]
                if bdt is None:
                    wt = w.T
                else:
                    wt = (_dot(bdt[:, g * 128:(g + 1) * 128], w, _NT) * _LOG2E).astype(bf16)
                wT[(t * D + g * 128) // 2:(t * D + (g + 1) * 128) // 2, :] = _pk(wt)

        def ln_x(i, dst, chunks=None):
            n = SB // NCH
            for c in (range(NCH) if chunks is None else chunks):
                dst[c * n // 2:(c + 1) * n // 2, :] = _pk(
                    _layernorm(x_v[rows_of(i, c, n), :].astype(f32)).astype(bf16))

        def proj(t, g, lo=0, n=SB):
            w = _upk(wT[(t * D + g * 128) // 2:(t * D + (g + 1) * 128) // 2, :])
            return _dot(w, _upk(xn_c[lo // 2:(lo + n) // 2, :]), _NT)

        def post_k(g, pk, first):
            out = []
            for hf in range(2):
                g4 = 2 * g + hf
                phik = _dual_softmax(pk[hf * 64:(hf + 1) * 64])
                zs = jnp.concatenate(
                    [functools.reduce(jnp.add, [r[:, j:j + 128] for j in range(0, r.shape[1], 128)])
                     for r in phik], axis=0)
                zacc[g4] = zs if first else zacc[g4] + zs
                out.append(_pack_feat(phik))
            return out

        def do_k(groups=range(G)):
            phiks = []
            for g in groups:
                phiks += post_k(g, proj(1, g), False)
            return phiks

        def do_q(i, groups=range(G)):
            for g in groups:
                pq = proj(0, g)
                for hf in range(2):
                    phiq[2 * g + hf, :, rows_of(i)] = _pack_feat(_dual_softmax(pq[hf * 64:(hf + 1) * 64]))

        def do_vkv(phiks, first):
            vTs = []
            for g in range(G):
                vT = proj(2, g)
                vTs += [vT[hf * 64:(hf + 1) * 64].astype(bf16) for hf in range(2)]
            for g4 in range(G4):
                kv = _dot(vTs[g4], _upk(phiks[g4]), _NT)
                kvacc[g4] = kv if first else kvacc[g4] + kv

        def finalize():
            r2 = lax.broadcasted_iota(i32, (64, 128), 0)
            c2 = lax.broadcasted_iota(i32, (64, 128), 1)
            kmask = (r2 // Dh) == ((c2 // 2) % 4)
            for g4 in range(G4):
                kvT[g4] = _pk(jnp.where(kmask, kvacc[g4], 0.0).astype(bf16))
                z = jnp.sum(zacc[g4], axis=-1, keepdims=True)
                zb[g4] = jnp.broadcast_to(z, (128, 128))

        def attn_o(i):
            os_ = []
            for g in range(G):
                parts = []
                for hf in range(2):
                    g4 = 2 * g + hf
                    pqi = phiq[g4, :, rows_of(i)]
                    numT = _dot(_upk(kvT[g4]), _upk(pqi))
                    zg = zb[g4]
                    den = None
                    for r in range(16):
                        m, pn = r % 8, r // 8
                        pf = pltpu.unpack_elementwise(pqi[m * 8:(m + 1) * 8], index=pn,
                                                      packed_dtype=bf16, unpacked_dtype=f32)
                        t = pf * jnp.concatenate([zg[r * 8:(r + 1) * 8]] * (SB // 128), axis=1)
                        den = t if den is None else den + t
                    den = den + pltpu.roll(den, 4, 0)
                    rd = _recip(den + 1e-6)
                    for h in range(4):
                        parts.append(numT[h * Dh:(h + 1) * Dh] * jnp.broadcast_to(rd[h:h + 1], (Dh, SB)))
                oT = jnp.concatenate(parts, axis=0)
                os_.append(oT.astype(bf16).T)
            return jnp.concatenate(os_, axis=1)

        def attn_out(i, o, hn_dst):
            h_v[rows_of(i), :] = x_v[rows_of(i), :].astype(f32) + _dot(o, wo_v[...])
            n = SB // NCH
            for c in range(NCH):
                hn_dst[c * n // 2:(c + 1) * n // 2, :] = _pk(
                    _layernorm(h_v[rows_of(i, c, n), :]).astype(bf16))

        def ffn1():
            a = _dot(_upk(hn_c[...]), w1_v[...]) + b1_v[...].astype(f32).reshape(1, F)
            a = jnp.maximum(a, 0.0)
            return (a * a).astype(bf16)

        def ffn2(i, a, c=0, n=SB):
            r = rows_of(i, c, n)
            out = h_v[r, :] + _dot(a, w2_v[...]) + b2_v[...].astype(f32).reshape(1, D)
            o_v[r, :] = out.astype(o_v.dtype)

        @pl.when(s == 0)
        def _():
            cp_phi.start()
            cp_wk(0).start()
            cp_x0(0).start()
            cp_wk(1).start()
            cp_x0(1).start()
            cp_w(0).start()
            cp_w(2).start()
            for b in range(1, NB):
                cp_x(b).start()
            for c in late:
                c.start()
            HB = SB // 2
            cp_phi.wait()
            bdt = build_bdt()
            cp_wk(0).wait()
            fold(1, bdt, (0, 1))
            cp_x0(0).wait()
            ln_x(0, xn_c, range(NCH // 2))
            ka = post_k(0, proj(1, 0, 0, HB), True)
            pk = proj(1, 1, 0, HB)
            cp_wk(1).wait()
            cp_x0(1).wait()
            fold(1, bdt, (2, 3))
            ka += post_k(1, pk, True)
            ln_x(0, xn_c, range(NCH // 2, NCH))
            for g in (2, 3):
                ka += post_k(g, proj(1, g, 0, HB), True)
            kb = []
            for g in range(G - 1):
                kb += post_k(g, proj(1, g, HB, HB), False)
            pk = proj(1, G - 1, HB, HB)
            cp_w(0).wait()
            fold(0, bdt)
            kb += post_k(G - 1, pk, False)
            phiks = [jnp.concatenate([u, v], axis=1) for u, v in zip(ka, kb)]
            cp_w(2).wait()
            cp_x(1).wait()
            fold(2, None)
            do_q(0)
            do_vkv(phiks, True)
            ln_x(1, xn_n)
            xn_c[...] = xn_n[...]

        @pl.when(s == 1)
        def _():
            for b in range(2, NB):
                cp_x(b).wait()
            late[0].wait()
            for b in range(1, NB - 1):
                phiks = do_k()
                do_q(b)
                do_vkv(phiks, False)
                ln_x(b + 1, xn_n)
                xn_c[...] = xn_n[...]
            phiks = do_k()
            do_vkv(phiks, False)
            do_q(NB - 1, (0,))
            finalize()
            o = attn_o(0)
            do_q(NB - 1, (1, 2))
            attn_out(0, o, hn_n)
            do_q(NB - 1, (3,))
            hn_c[...] = hn_n[...]

        @pl.when(s == 2)
        def _():
            for c in late[1:]:
                c.wait()

        @pl.when((s >= 2) & (s < NB + 1))
        def _():
            i = s - 2
            o = attn_o(i + 1)
            a = ffn1()
            attn_out(i + 1, o, hn_n)
            ffn2(i, a)
            hn_c[...] = hn_n[...]
            for b in range(NB - 1):
                @pl.when(i == b)
                def _():
                    cp_o(b).start()

        @pl.when(s == NB + 1)
        def _():
            a = ffn1()
            n = SB // NO
            for c in range(NO):
                ffn2(NB - 1, a[c * n:(c + 1) * n], c, n)
                cp_o(NB - 1, c, n).start()
            cp(o_v, o_hbm, SEM_OUT).wait()

    x2 = A_x.reshape(S, D)
    wphi2 = jnp.transpose(A_w_phi, (1, 2, 0)).reshape(Dh * Dh, H)
    any_spec = pl.BlockSpec(memory_space=pl.ANY)
    out = pl.pallas_call(
        kernel,
        grid=(NB + 2,),
        in_specs=[any_spec] * 8,
        out_specs=any_spec,
        out_shape=jax.ShapeDtypeStruct((S, D), A_x.dtype),
        scratch_shapes=[
            pltpu.VMEM((S, D), bf16),
            pltpu.VMEM((D, 3 * D), bf16),
            pltpu.VMEM((Dh * Dh, H), bf16),
            pltpu.VMEM((D, D), bf16),
            pltpu.VMEM((D, F), bf16),
            pltpu.VMEM((F,), bf16),
            pltpu.VMEM((F, D), bf16),
            pltpu.VMEM((D,), bf16),
            pltpu.VMEM((S, D), bf16),
            pltpu.VMEM((3 * D // 2, D), i32),
            pltpu.VMEM((SB // 2, D), i32),
            pltpu.VMEM((SB // 2, D), i32),
            pltpu.VMEM((S, D), f32),
            pltpu.VMEM((G4, 64, S), i32),
            pltpu.VMEM((G4, 64, 128), f32),
            pltpu.VMEM((G4, 128, 128), f32),
            pltpu.VMEM((G4, 32, 128), i32),
            pltpu.VMEM((G4, 128, 128), f32),
            pltpu.SemaphoreType.DMA((9,)),
        ],
        compiler_params=pltpu.CompilerParams(
            dimension_semantics=("arbitrary",),
            vmem_limit_bytes=100 * 1024 * 1024,
        ),
    )(x2, A_wqkv, wphi2, A_wo, B_w1, B_b1, B_w2, B_b2)
    return out.reshape(B, S, D)
```
